```python
import os as _os
_os.environ.setdefault("JAX_PLATFORMS", "cpu")
import jax
import jax.numpy as jnp

def _softmax(x, axis=-1):
    return jax.nn.softmax(x, axis=axis)
def _gelu(x):
    return jax.nn.gelu(x, approximate=True)
def _silu(x):
    return jax.nn.silu(x)
def _sigmoid(x):
    return jax.nn.sigmoid(x)
def _layernorm(x, axis=-1, eps=1e-5):
    m = jnp.mean(x, axis=axis, keepdims=True)
    v = jnp.var(x, axis=axis, keepdims=True)
    return (x - m) / jnp.sqrt(v + eps)
def _scatter_add(tgt, idx, src, axis=0):
    return tgt.at[idx].add(src)
def _segment_sum(src, seg, n):
    return jax.ops.segment_sum(src, seg, n)
class _Rng:
    def __init__(self, key):
        self._k = key
    def _next(self):
        self._k, sub = jax.random.split(self._k)
        return sub
    def normal(self, shape):
        return jax.random.normal(self._next(), shape, dtype=jnp.bfloat16)
    def randint(self, lo, hi, shape):
        return jax.random.randint(self._next(), shape, lo, hi, dtype=jnp.int32)
    def uniform(self, shape, lo=0.0, hi=1.0):
        return jax.random.uniform(self._next(), shape, jnp.bfloat16, lo, hi)
    def permutation(self, n):
        return jax.random.permutation(self._next(), n)


kernel_name = 'gated_mix__linear_kernel_hedgehog__glu_gated_bilinear__prompt'

def setup_inputs():
    _rng = _Rng(jax.random.key(int.from_bytes(__import__("os").urandom(4), "little")))
    _w = (lambda a: (lambda t: t.astype(jnp.bfloat16) if jnp.issubdtype(t.dtype, jnp.floating) else t)(jnp.asarray(a)))
    def _A_setup():
        B, S, D, H = 1, 2048, 512, 32
        Dh = D // H
        return {
            "x": _w((lambda *s: _rng.normal(s) * 0.05)(B, S, D)),
            "wqkv": _w((lambda *s: _rng.normal(s) * 0.8)(D, 3 * D)),
            "w_phi": _w((lambda *s: _rng.normal(s) * 0.8)(H, Dh, Dh) * (Dh ** -0.5)),
            "wo": _w((lambda *s: _rng.normal(s) * 0.05)(D, D)),
        }
    _A_in = _A_setup()

    def _B_setup():
        B, S, D, F = 1, 2048, 512, 1792
        return {
            "x": _w((lambda *s: _rng.normal(s) * 0.05)(B, S, D)),
            "w_gate": _w((lambda *s: _rng.normal(s) * 1.6)(D, F) * (D ** -0.5)),
            "w_up": _w((lambda *s: _rng.normal(s) * 1.6)(D, F) * (D ** -0.5)),
            "w_down": _w((lambda *s: _rng.normal(s) * 1.6)(F, D) * (F ** -0.5)),
        }
    _B_in = _B_setup()

    return {
        "A_x": _A_in["x"],
        "A_wqkv": _A_in["wqkv"],
        "A_w_phi": _A_in["w_phi"],
        "A_wo": _A_in["wo"],
        "B_x": _B_in["x"],
        "B_w_gate": _B_in["w_gate"],
        "B_w_up": _B_in["w_up"],
        "B_w_down": _B_in["w_down"],
        "gate_w": _w((lambda *s: _rng.normal(s) * 0.05)(512) * 16.0),
    }

def reference(A_x, A_wqkv, A_w_phi, A_wo, B_x, B_w_gate, B_w_up, B_w_down, gate_w):
    def _A_ref(x, wqkv, w_phi, wo):
        B, S, D = x.shape
        H = 32; Dh = D // H
        qkv = (lambda x, *d: x.transpose(*d))((x @ wqkv).reshape(B, S, 3, H, Dh), 2, 0, 3, 1, 4)
        q, k, v = qkv[0], qkv[1], qkv[2]
        pq = jnp.einsum("bhsd,hdf->bhsf", q, w_phi)
        pk = jnp.einsum("bhsd,hdf->bhsf", k, w_phi)
        phi_q = jnp.concatenate([_softmax(pq, axis=-1), _softmax(-pq, axis=-1)], axis=-1)
        phi_k = jnp.concatenate([_softmax(pk, axis=-1), _softmax(-pk, axis=-1)], axis=-1)
        kv = jnp.einsum("bhsf,bhsd->bhfd", phi_k, v)
        z  = jnp.einsum("bhsf->bhf", phi_k)
        num = jnp.einsum("bhqf,bhfd->bhqd", phi_q, kv)
        den = jnp.einsum("bhqf,bhf->bhq", phi_q, z)[..., None] + 1e-6
        o = num / den
        return (lambda x, *d: x.transpose(*d))(o, 0, 2, 1, 3).reshape(B, S, D) @ wo

    def _B_ref(x, w_gate, w_up, w_down):
        g = jnp.einsum("bsd,df->bsf", x, w_gate)
        u = jnp.einsum("bsd,df->bsf", x, w_up)
        h = g * u
        return jnp.einsum("bsf,fd->bsd", h, w_down)

    x = A_x
    g = _sigmoid((x * gate_w).sum(-1, keepdims=True))
    a = _A_ref(x, A_wqkv, A_w_phi, A_wo)
    b = _B_ref(x, B_w_gate, B_w_up, B_w_down)
    return g * a + (1 - g) * b
```

```python
import functools
import numpy as np
import jax
import jax.numpy as jnp
from jax import lax
import jax.experimental.pallas as pl
import jax.experimental.pallas.tpu as pltpu

S, D, H, DH, F = 2048, 512, 32, 16, 1792
G = 4
NT = (((1,), (1,)), ((), ()))
NN = (((1,), (0,)), ((), ()))
LOG2E = 1.4426950408889634
f32, bf16 = jnp.float32, jnp.bfloat16


def _dual_softmax(p):
    T = p.shape[-1]
    p3 = p.reshape(16, 8, T)
    mx = jnp.max(p3, axis=0, keepdims=True)
    mn = jnp.min(p3, axis=0, keepdims=True)
    ep = jnp.exp2(p3 - mx)
    en = jnp.exp2(mn - p3)
    rp = 1.0 / jnp.sum(ep, axis=0, keepdims=True)
    rn = 1.0 / jnp.sum(en, axis=0, keepdims=True)
    return (ep * rp), (en * rn)


def make(T1=256, T2=256, FC=256, interpret=False):
    N1, N2 = S // T1, S // T2

    def kernel(x_h, wqkv_h, wphi_h, wo_h, wg_h, wu_h, wd_h, gw_h, o_h,
               x_v, wqkv_v, wphi_v, wo_v, wg_v, wu_v, wd_v, gw_v, o_v,
               wT_v, kv_v, z_v, kvb_v, semx, semw, semo):
        def xcopy(i):
            r = pl.ds(pl.multiple_of(i * T1, T1), T1)
            return pltpu.make_async_copy(x_h.at[r], x_v.at[r], semx.at[i])

        def ocopy(i):
            r = pl.ds(pl.multiple_of(i * T2, T2), T2)
            return pltpu.make_async_copy(o_v.at[r], o_h.at[r], semo.at[i])

        c_phi = pltpu.make_async_copy(wphi_h, wphi_v, semw.at[0])
        c_kv = pltpu.make_async_copy(wqkv_h.at[:, pl.ds(D, 2 * D)], wqkv_v.at[:, pl.ds(D, 2 * D)], semw.at[1])
        c_q = pltpu.make_async_copy(wqkv_h.at[:, pl.ds(0, D)], wqkv_v.at[:, pl.ds(0, D)], semw.at[2])
        c_rest = [pltpu.make_async_copy(a, b, semw.at[3 + n]) for n, (a, b) in enumerate(
            [(gw_h, gw_v), (wg_h, wg_v), (wu_h, wu_v), (wd_h, wd_v), (wo_h, wo_v)])]
        c_phi.start()
        c_kv.start()
        for i in range(N1):
            xcopy(i).start()
        c_q.start()
        for c in c_rest:
            c.start()

        r16 = lax.broadcasted_iota(jnp.int32, (128, 16), 0)
        c16 = lax.broadcasted_iota(jnp.int32, (128, 16), 1)
        E = ((r16 // 8) == c16).astype(bf16)
        rr = lax.broadcasted_iota(jnp.int32, (128, 128), 0)
        cc = lax.broadcasted_iota(jnp.int32, (128, 128), 1)
        bdmask = (rr % 8) == (cc // 16)

        c_phi.wait()

        def bdt(g):
            t = lax.dot_general(E, wphi_v[pl.ds(g * 128, 128), :], NT, preferred_element_type=f32)
            return jnp.where(bdmask, t, 0.0).astype(bf16)

        def prep(base_in, base_out):
            for g in range(G):
                w = wqkv_v[:, pl.ds(base_in + g * 128, 128)]
                t = lax.dot_general(bdt(g), w, NT, preferred_element_type=f32)
                wT_v[pl.ds(base_out + g * 128, 128), :] = (t * LOG2E).astype(bf16)

        c_kv.wait()
        prep(D, D)
        kv_v[...] = jnp.zeros(kv_v.shape, f32)
        z_v[...] = jnp.zeros(z_v.shape, f32)

        def body1(i, carry):
            xcopy(i).wait()
            x = x_v[pl.ds(pl.multiple_of(i * T1, T1), T1), :]
            pk = lax.dot_general(wT_v[pl.ds(D, D), :], x, NT, preferred_element_type=f32)
            v = lax.dot_general(x, wqkv_v[:, pl.ds(2 * D, D)], NN, preferred_element_type=f32).astype(bf16)
            for g in range(G):
                pp, pn = _dual_softmax(pk[g * 128:(g + 1) * 128])
                ph = jnp.concatenate([pp.reshape(128, T1), pn.reshape(128, T1)], axis=0)
                zz = ph[:, 0:128]
                for j in range(1, T1 // 128):
                    zz = zz + ph[:, j * 128:(j + 1) * 128]
                z_v[g] += zz
                kv_v[g] += lax.dot_general(ph.astype(bf16), v[:, g * 128:(g + 1) * 128], NN, preferred_element_type=f32)
            return carry

        lax.fori_loop(0, N1, body1, 0)

        c_q.wait()
        prep(0, 0)
        r2 = lax.broadcasted_iota(jnp.int32, (128, 256), 0)
        c2 = lax.broadcasted_iota(jnp.int32, (128, 256), 1)
        m2 = (r2 // 16) == (c2 % 8)
        for g in range(G):
            kvb_v[g] = jnp.where(m2, kv_v[g].T, 0.0).astype(bf16)
            z_v[g] = jnp.broadcast_to(jnp.sum(z_v[g], axis=1, keepdims=True), (256, 128))
        for c in c_rest:
            c.wait()

        def body2(i, carry):
            x = x_v[pl.ds(pl.multiple_of(i * T2, T2), T2), :]
            pq = lax.dot_general(wT_v[pl.ds(0, D), :], x, NT, preferred_element_type=f32)
            gl = jnp.sum(x.astype(f32) * gw_v[...].astype(f32), axis=1, keepdims=True)
            gate = jax.nn.sigmoid(gl)
            os_ = []
            for g in range(G):
                pp, pn = _dual_softmax(pq[g * 128:(g + 1) * 128])
                z = z_v[g]
                z = jnp.concatenate([z] * (T2 // 128), axis=1)
                den = jnp.sum(pp * z[0:128].reshape(16, 8, T2) + pn * z[128:256].reshape(16, 8, T2), axis=0) + 1e-6
                ph = jnp.concatenate([pp.reshape(128, T2), pn.reshape(128, T2)], axis=0).astype(bf16)
                num = lax.dot_general(kvb_v[g], ph, NN, preferred_element_type=f32)
                r = 1.0 / den
                rb = jnp.broadcast_to(r[:, None, :], (8, 16, T2)).reshape(128, T2)
                os_.append((num * rb).astype(bf16))
            oT = jnp.concatenate(os_, axis=0)
            o = oT.T
            a = lax.dot_general(o, wo_v[...], NN, preferred_element_type=f32)
            b = None
            for c in range(F // FC):
                gg = lax.dot_general(x, wg_v[:, pl.ds(c * FC, FC)], NN, preferred_element_type=f32)
                uu = lax.dot_general(x, wu_v[:, pl.ds(c * FC, FC)], NN, preferred_element_type=f32)
                h = (gg * uu).astype(bf16)
                t = lax.dot_general(h, wd_v[pl.ds(c * FC, FC), :], NN, preferred_element_type=f32)
                b = t if b is None else b + t
            o_v[pl.ds(pl.multiple_of(i * T2, T2), T2), :] = (gate * a + (1.0 - gate) * b).astype(bf16)
            ocopy(i).start()
            return carry

        lax.fori_loop(0, N2, body2, 0)
        for i in range(N2):
            ocopy(i).wait()

    @jax.jit
    def fn(A_x, A_wqkv, A_w_phi, A_wo, B_x, B_w_gate, B_w_up, B_w_down, gate_w):
        any_ = pl.BlockSpec(memory_space=pl.ANY)
        out = pl.pallas_call(
            kernel,
            out_shape=jax.ShapeDtypeStruct((S, D), bf16),
            in_specs=[any_] * 8,
            out_specs=any_,
            scratch_shapes=[
                pltpu.VMEM((S, D), bf16), pltpu.VMEM((D, 3 * D), bf16), pltpu.VMEM((D, DH), bf16),
                pltpu.VMEM((D, D), bf16), pltpu.VMEM((D, F), bf16), pltpu.VMEM((D, F), bf16),
                pltpu.VMEM((F, D), bf16), pltpu.VMEM((1, D), bf16), pltpu.VMEM((S, D), bf16),
                pltpu.VMEM((2 * D, D), bf16), pltpu.VMEM((G, 256, 128), f32), pltpu.VMEM((G, 256, 128), f32),
                pltpu.VMEM((G, 128, 256), bf16),
                pltpu.SemaphoreType.DMA((N1,)), pltpu.SemaphoreType.DMA((8,)), pltpu.SemaphoreType.DMA((N2,)),
            ],
            compiler_params=pltpu.CompilerParams(vmem_limit_bytes=100 * 1024 * 1024),
            interpret=interpret,
        )(A_x.reshape(S, D), A_wqkv, A_w_phi.reshape(D, DH), A_wo, B_w_gate, B_w_up, B_w_down, gate_w.reshape(1, D))
        return out.reshape(1, S, D)
    return fn


_IMPL = make(T1=512,T2=512,FC=896)


def pallas_gated_mix__linear_kernel_hedgehog__glu_gated_bilinear__prompt_kernel(
    A_x, A_wqkv, A_w_phi, A_wo, B_x, B_w_gate, B_w_up, B_w_down, gate_w):
    return _IMPL(A_x, A_wqkv, A_w_phi, A_wo, B_x, B_w_gate, B_w_up, B_w_down, gate_w)
```

```python
import functools
import numpy as np
import jax
import jax.numpy as jnp
from jax import lax
import jax.experimental.pallas as pl
import jax.experimental.pallas.tpu as pltpu

S, D, H, DH, F = 2048, 512, 32, 16, 1792
G = 4
NT = (((1,), (1,)), ((), ()))
NN = (((1,), (0,)), ((), ()))
LOG2E = 1.4426950408889634
f32, bf16 = jnp.float32, jnp.bfloat16


def _dual_softmax(p):
    T = p.shape[-1]
    p3 = p.reshape(16, 8, T)
    mx = jnp.max(p3, axis=0, keepdims=True)
    mn = jnp.min(p3, axis=0, keepdims=True)
    ep = jnp.exp2(p3 - mx)
    en = jnp.exp2(mn - p3)
    rp = 1.0 / jnp.sum(ep, axis=0, keepdims=True)
    rn = 1.0 / jnp.sum(en, axis=0, keepdims=True)
    return (ep * rp), (en * rn)


def make(T1=256, T2=256, FC=256, stag=1, interpret=False):
    N1, N2 = S // T1, S // T2

    def kernel(x_h, wqkv_h, wphi_h, wo_h, wg_h, wu_h, wd_h, gw_h, o_h,
               x_v, wqkv_v, wphi_v, wo_v, wg_v, wu_v, wd_v, gw_v, o_v,
               wT_v, kv_v, z_v, kvb_v, semx, semw, semo):
        def xcopy(i):
            r = pl.ds(pl.multiple_of(i * T1, T1), T1)
            return pltpu.make_async_copy(x_h.at[r], x_v.at[r], semx.at[i])

        def ocopy(i):
            r = pl.ds(pl.multiple_of(i * T2, T2), T2)
            return pltpu.make_async_copy(o_v.at[r], o_h.at[r], semo.at[i])

        c_phi = pltpu.make_async_copy(wphi_h, wphi_v, semw.at[0])
        c_kv = pltpu.make_async_copy(wqkv_h.at[:, pl.ds(D, D)], wqkv_v.at[:, pl.ds(D, D)], semw.at[1])
        c_v = pltpu.make_async_copy(wqkv_h.at[:, pl.ds(2 * D, D)], wqkv_v.at[:, pl.ds(2 * D, D)], semw.at[8])
        c_q = pltpu.make_async_copy(wqkv_h.at[:, pl.ds(0, D)], wqkv_v.at[:, pl.ds(0, D)], semw.at[2])
        c_rest = [pltpu.make_async_copy(a, b, semw.at[3 + n]) for n, (a, b) in enumerate(
            [(gw_h, gw_v), (wg_h, wg_v), (wu_h, wu_v), (wd_h, wd_v), (wo_h, wo_v)])]
        c_phi.start()
        c_kv.start()
        xcopy(0).start()
        c_v.start()
        def rest():
            for i in range(1, N1):
                xcopy(i).start()
            c_q.start()
            for c in c_rest:
                c.start()
        if stag == 0:
            rest()

        def iota(shape, d):
            return lax.broadcasted_iota(jnp.int32, shape, d)
        r = iota((D, H), 0)
        A = (((r // 128) * 8 + r % 8) == iota((D, H), 1)).astype(bf16)
        sel = ((iota((256, 128), 0) // 16) == (iota((256, 128), 1) % 16)).astype(bf16)
        m1 = ((iota((D, 256), 0) % 128) // 8) == (iota((D, 256), 1) % 16)
        m3 = (iota((D, 128), 0) % 8) == (iota((D, 128), 1) // 16)
        c_phi.wait()
        t = lax.dot_general(A, wphi_v[...], NT, preferred_element_type=f32)
        t = jnp.where(m1, t, 0.0).astype(bf16)
        t = lax.dot_general(t, sel, NN, preferred_element_type=f32)
        bd = jnp.where(m3, t, 0.0).astype(bf16)

        def bdt(g):
            return bd[g * 128:(g + 1) * 128]

        def prep(base_in, base_out):
            for g in range(G):
                w = wqkv_v[:, pl.ds(base_in + g * 128, 128)]
                t = lax.dot_general(bdt(g), w, NT, preferred_element_type=f32)
                wT_v[pl.ds(base_out + g * 128, 128), :] = (t * LOG2E).astype(bf16)

        c_kv.wait()
        if stag == 1:
            rest()
        prep(D, D)
        kv_v[...] = jnp.zeros(kv_v.shape, f32)
        z_v[...] = jnp.zeros(z_v.shape, f32)

        c_v.wait()
        if stag == 2:
            rest()

        def body1(i, carry):
            xcopy(i).wait()
            x = x_v[pl.ds(pl.multiple_of(i * T1, T1), T1), :]
            pk = lax.dot_general(wT_v[pl.ds(D, D), :], x, NT, preferred_element_type=f32)
            v = lax.dot_general(x, wqkv_v[:, pl.ds(2 * D, D)], NN, preferred_element_type=f32).astype(bf16)
            for g in range(G):
                pp, pn = _dual_softmax(pk[g * 128:(g + 1) * 128])
                ph = jnp.concatenate([pp.reshape(128, T1), pn.reshape(128, T1)], axis=0)
                zz = ph[:, 0:128]
                for j in range(1, T1 // 128):
                    zz = zz + ph[:, j * 128:(j + 1) * 128]
                z_v[g] += zz
                kv_v[g] += lax.dot_general(ph.astype(bf16), v[:, g * 128:(g + 1) * 128], NN, preferred_element_type=f32)
            return carry

        lax.fori_loop(0, N1, body1, 0)

        c_q.wait()
        prep(0, 0)
        r2 = lax.broadcasted_iota(jnp.int32, (128, 256), 0)
        c2 = lax.broadcasted_iota(jnp.int32, (128, 256), 1)
        m2 = (r2 // 16) == (c2 % 8)
        for g in range(G):
            kvb_v[g] = jnp.where(m2, kv_v[g].T, 0.0).astype(bf16)
            z_v[g] = jnp.broadcast_to(jnp.sum(z_v[g], axis=1, keepdims=True), (256, 128))
        for c in c_rest:
            c.wait()

        def body2(i, carry):
            x = x_v[pl.ds(pl.multiple_of(i * T2, T2), T2), :]
            pq = lax.dot_general(wT_v[pl.ds(0, D), :], x, NT, preferred_element_type=f32)
            gl = jnp.sum(x.astype(f32) * gw_v[...].astype(f32).reshape(1, D), axis=1, keepdims=True)
            gate = jax.nn.sigmoid(gl)
            os_ = []
            for g in range(G):
                pp, pn = _dual_softmax(pq[g * 128:(g + 1) * 128])
                z = z_v[g]
                z = jnp.concatenate([z] * (T2 // 128), axis=1)
                den = jnp.sum(pp * z[0:128].reshape(16, 8, T2) + pn * z[128:256].reshape(16, 8, T2), axis=0) + 1e-6
                ph = jnp.concatenate([pp.reshape(128, T2), pn.reshape(128, T2)], axis=0).astype(bf16)
                num = lax.dot_general(kvb_v[g], ph, NN, preferred_element_type=f32)
                r = 1.0 / den
                rb = jnp.broadcast_to(r[:, None, :], (8, 16, T2)).reshape(128, T2)
                os_.append((num * rb).astype(bf16))
            oT = jnp.concatenate(os_, axis=0)
            o = oT.T
            a = lax.dot_general(o, wo_v[...], NN, preferred_element_type=f32)
            b = None
            for c in range(F // FC):
                gg = lax.dot_general(x, wg_v[:, pl.ds(c * FC, FC)], NN, preferred_element_type=f32)
                uu = lax.dot_general(x, wu_v[:, pl.ds(c * FC, FC)], NN, preferred_element_type=f32)
                h = (gg * uu).astype(bf16)
                t = lax.dot_general(h, wd_v[pl.ds(c * FC, FC), :], NN, preferred_element_type=f32)
                b = t if b is None else b + t
            o_v[pl.ds(pl.multiple_of(i * T2, T2), T2), :] = (gate * a + (1.0 - gate) * b).astype(bf16)
            ocopy(i).start()
            return carry

        lax.fori_loop(0, N2, body2, 0)
        for i in range(N2):
            ocopy(i).wait()

    @jax.jit
    def fn(A_x, A_wqkv, A_w_phi, A_wo, B_x, B_w_gate, B_w_up, B_w_down, gate_w):
        any_ = pl.BlockSpec(memory_space=pl.ANY)
        out = pl.pallas_call(
            kernel,
            out_shape=jax.ShapeDtypeStruct((S, D), bf16),
            in_specs=[any_] * 8,
            out_specs=any_,
            scratch_shapes=[
                pltpu.VMEM((S, D), bf16), pltpu.VMEM((D, 3 * D), bf16), pltpu.VMEM((DH * DH, H), bf16),
                pltpu.VMEM((D, D), bf16), pltpu.VMEM((D, F), bf16), pltpu.VMEM((D, F), bf16),
                pltpu.VMEM((F, D), bf16), pltpu.VMEM((D,), bf16), pltpu.VMEM((S, D), bf16),
                pltpu.VMEM((2 * D, D), bf16), pltpu.VMEM((G, 256, 128), f32), pltpu.VMEM((G, 256, 128), f32),
                pltpu.VMEM((G, 128, 256), bf16),
                pltpu.SemaphoreType.DMA((N1,)), pltpu.SemaphoreType.DMA((9,)), pltpu.SemaphoreType.DMA((N2,)),
            ],
            compiler_params=pltpu.CompilerParams(vmem_limit_bytes=100 * 1024 * 1024),
            interpret=interpret,
        )(A_x.reshape(S, D), A_wqkv, A_w_phi.transpose(1, 2, 0).reshape(DH * DH, H), A_wo, B_w_gate, B_w_up, B_w_down, gate_w)
        return out.reshape(1, S, D)
    return fn


_IMPL = make(T1=256, T2=512, FC=896)


@jax.jit
def pallas_gated_mix__linear_kernel_hedgehog__glu_gated_bilinear__prompt_kernel(
    A_x, A_wqkv, A_w_phi, A_wo, B_x, B_w_gate, B_w_up, B_w_down, gate_w):
    return _IMPL(A_x, A_wqkv, A_w_phi, A_wo, B_x, B_w_gate, B_w_up, B_w_down, gate_w)
```
